```python
import jax
import jax.numpy as jnp

def _softmax(x, axis=-1):
    return jax.nn.softmax(x, axis=axis)
def _gelu(x):
    return jax.nn.gelu(x, approximate=True)
def _silu(x):
    return jax.nn.silu(x)
def _sigmoid(x):
    return jax.nn.sigmoid(x)
def _layernorm(x, axis=-1, eps=1e-5):
    m = jnp.mean(x, axis=axis, keepdims=True)
    v = jnp.var(x, axis=axis, keepdims=True)
    return (x - m) / jnp.sqrt(v + eps)
def _scatter_add(tgt, idx, src, axis=0):
    return tgt.at[idx].add(src)
def _segment_sum(src, seg, n):
    return jax.ops.segment_sum(src, seg, n)
class _Rng:
    def __init__(self, key):
        self._k = key
    def _next(self):
        self._k, sub = jax.random.split(self._k)
        return sub
    def normal(self, shape):
        return jax.random.normal(self._next(), shape, dtype=jnp.bfloat16)
    def randint(self, lo, hi, shape):
        return jax.random.randint(self._next(), shape, lo, hi, dtype=jnp.int32)
    def uniform(self, shape, lo=0.0, hi=1.0):
        return jax.random.uniform(self._next(), shape, jnp.bfloat16, lo, hi)
    def permutation(self, n):
        return jax.random.permutation(self._next(), n)


kernel_name = 'concat_heads__gqa_block_cached__compressed_kv_cla__decode'

def setup_inputs():
    _rng = _Rng(jax.random.key(int.from_bytes(__import__("os").urandom(4), "little")))
    _w = (lambda a: (lambda t: t.astype(jnp.bfloat16) if jnp.issubdtype(t.dtype, jnp.floating) else t)(jnp.asarray(a)))
    def _A_setup():
        B, Sq, D = 2, 1, 512
        Hq, Hkv, Sk, Dh = 32, 32, 8192, 128
        assert Hq % Hkv == 0, (Hq, Hkv)
        return {
            "x": _w((lambda *s: _rng.normal(s) * 0.05)(B, Sq, D)),
            "k_cache": _w((lambda *s: _rng.normal(s) * 0.05)(B, Hkv, Sk, Dh)),
            "v_cache": _w((lambda *s: _rng.normal(s) * 0.05)(B, Hkv, Sk, Dh)),
            "wq": _w((lambda *s: _rng.normal(s) * 0.05)(D, Hq * Dh) * (D ** -0.5)),
            "wo": _w((lambda *s: _rng.normal(s) * 0.05)(Hq * Dh, D) * ((Hq * Dh) ** -0.5)),
        }
    _A_in = _A_setup()

    def _B_setup():
        B, H, Sq, Sk, D, M = 2, 32, 1, 8192, 128, 512
        Dc = 4 * D
        return {
            "x": _w((lambda *s: _rng.normal(s) * 0.05)(B, Sq, M)),
            "c_kv": _w((lambda *s: _rng.normal(s) * 0.05)(B, Sk, Dc)),
            "w_q": _w((lambda *s: _rng.normal(s) * 0.05)(M, H, D) * (M ** -0.5)),
            "w_uk": _w((lambda *s: _rng.normal(s) * 0.05)(Dc, H, D) * (Dc ** -0.5)),
            "w_uv": _w((lambda *s: _rng.normal(s) * 0.05)(Dc, H, D) * (Dc ** -0.5)),
            "w_o": _w((lambda *s: _rng.normal(s) * 0.05)(H, D, M) * ((H * D) ** -0.5)),
        }
    _B_in = _B_setup()

    return {
        "A_x": _A_in["x"],
        "A_k_cache": _A_in["k_cache"],
        "A_v_cache": _A_in["v_cache"],
        "A_wq": _A_in["wq"],
        "A_wo": _A_in["wo"],
        "B_x": _B_in["x"],
        "B_c_kv": _B_in["c_kv"],
        "B_w_q": _B_in["w_q"],
        "B_w_uk": _B_in["w_uk"],
        "B_w_uv": _B_in["w_uv"],
        "B_w_o": _B_in["w_o"],
    }

def reference(A_x, A_k_cache, A_v_cache, A_wq, A_wo, B_x, B_c_kv, B_w_q, B_w_uk, B_w_uv, B_w_o):
    def _A_ref(x, k_cache, v_cache, wq, wo):
        B, Sq, D = x.shape
        Hq, Dh = 32, 128
        Hkv = k_cache.shape[1]
        rep = Hq // Hkv
        q = (lambda x, *d: x.transpose(*d))((x @ wq).reshape(B, Sq, Hq, Dh), 0, 2, 1, 3)
        k = jnp.repeat(k_cache, rep, axis=1)
        v = jnp.repeat(v_cache, rep, axis=1)
        scores = jnp.einsum("bhqd,bhkd->bhqk", q, k) * (Dh ** -0.5)
        p = _softmax(scores, axis=-1)
        o = jnp.einsum("bhqk,bhkd->bhqd", p, v)
        return (lambda x, *d: x.transpose(*d))(o, 0, 2, 1, 3).reshape(B, Sq, Hq * Dh) @ wo

    def _B_ref(x, c_kv, w_q, w_uk, w_uv, w_o):
        B, Sq, M = x.shape[0], x.shape[1], x.shape[2]
        Sk = c_kv.shape[1]
        H, D = w_q.shape[1], w_q.shape[2]
        q = jnp.einsum("bqm,mhd->bhqd", x, w_q)
        k = jnp.einsum("bkc,chd->bhkd", c_kv, w_uk)
        v = jnp.einsum("bkc,chd->bhkd", c_kv, w_uv)
        scores = jnp.einsum("bhqd,bhkd->bhqk", q, k) * (D ** -0.5)
        off = Sk - Sq
        qi = jnp.arange(Sq)[:, None]
        kj = jnp.arange(Sk)[None, :]
        cmask = kj <= (qi + off)
        scores = jnp.where(cmask[None, None], scores, -1e9)
        p = _softmax(scores, axis=-1)
        ctx = jnp.einsum("bhqk,bhkd->bhqd", p, v)
        return jnp.einsum("bhqd,hdm->bqm", ctx, w_o)

    a = _A_ref(A_x, A_k_cache, A_v_cache, A_wq, A_wo)
    b = _B_ref(B_x, B_c_kv, B_w_q, B_w_uk, B_w_uv, B_w_o)
    return jnp.concatenate([a, b], axis=-1)
```

```python
import jax
import jax.numpy as jnp
from jax import lax
import jax.experimental.pallas as pl
import jax.experimental.pallas.tpu as pltpu

DEPTH = 4
VMEM_LIMIT = 100 * 1024 * 1024

_NT = (((1,), (1,)), ((), ()))


def _kernel(
    ax_hbm, k_hbm, v_hbm, awq_hbm, awo_hbm,
    bx_hbm, ckv_hbm, bwq_hbm, bwuk_hbm, bwuv_hbm, bwo_hbm,
    out_ref,
    ax_v, bx_v, awq_v, awo_v, ckv_v, bwq_v, bwuk_v, bwuv_v, bwo_v,
    kbuf, vbuf, q_scr, rsem, ksem, vsem,
    *, nb, nh, dh, depth,
):
    f32, bf16 = jnp.float32, jnp.bfloat16
    nsteps = nb * nh
    d_model = ax_v.shape[-1]

    res = {}
    order = [
        ("bx", bx_hbm, bx_v), ("ax", ax_hbm, ax_v),
        ("bwq", bwq_hbm, bwq_v), ("bwuk", bwuk_hbm, bwuk_v),
    ]
    for b in range(nb):
        order.append((f"ckv{b}", ckv_hbm.at[b], ckv_v.at[b]))
    order += [
        ("bwuv", bwuv_hbm, bwuv_v), ("bwo", bwo_hbm, bwo_v),
        ("awq", awq_hbm, awq_v),
    ]
    for i, (name, src, dst) in enumerate(order):
        res[name] = pltpu.make_async_copy(src, dst, rsem.at[i])
    res["awo"] = pltpu.make_async_copy(awo_hbm, awo_v, rsem.at[len(order)])

    def k_copy(i, slot):
        return pltpu.make_async_copy(
            k_hbm.at[i % nb, i // nb], kbuf.at[slot], ksem.at[slot])

    def v_copy(i, slot):
        return pltpu.make_async_copy(
            v_hbm.at[i % nb, i // nb], vbuf.at[slot], vsem.at[slot])

    for name, _, _ in order:
        res[name].start()
    k_copy(0, 0).start()
    v_copy(0, 0).start()
    res["awo"].start()
    for i in range(1, depth):
        k_copy(i, i).start()
        v_copy(i, i).start()

    row8 = lax.broadcasted_iota(jnp.int32, (8, d_model), 0)

    def rows_of(x_v):
        x = jnp.zeros((8, d_model), f32)
        for b in range(nb):
            x = jnp.where(row8 == b, x_v[b].astype(f32), x)
        return x.astype(bf16)

    scale = dh ** -0.5

    hd = nh * dh
    rows = lax.broadcasted_iota(jnp.int32, (nb * nh, hd), 0)
    lanes = lax.broadcasted_iota(jnp.int32, (nb * nh, hd), 1)
    diag = (rows % nh) == (lanes // dh)

    res["bx"].wait()
    xb = rows_of(bx_v)
    res["bwq"].wait()
    qb = jnp.dot(xb, bwq_v[...].reshape(d_model, hd),
                 preferred_element_type=f32)
    qb = qb.astype(bf16).astype(f32)
    q_bd = jnp.concatenate(
        [jnp.broadcast_to(qb[b:b + 1], (nh, hd)) for b in range(nb)], axis=0)
    q_bd = jnp.where(diag, q_bd, 0.0).astype(bf16)
    res["bwuk"].wait()
    dc = bwuk_v.shape[0]
    qlat = lax.dot_general(q_bd, bwuk_v[...].reshape(dc, hd), _NT,
                           preferred_element_type=f32)
    qlat = (qlat * scale).astype(bf16)

    ctx_parts = []
    for b in range(nb):
        res[f"ckv{b}"].wait()
        ckv = ckv_v[b]
        s = lax.dot_general(qlat[b * nh:(b + 1) * nh], ckv, _NT,
                            preferred_element_type=f32)
        m = jnp.max(s, axis=1, keepdims=True)
        p = jnp.exp(s - m)
        l = jnp.sum(p, axis=1, keepdims=True)
        c = jnp.dot(p.astype(bf16), ckv, preferred_element_type=f32)
        ctx_parts.append((c / l).astype(bf16))
    ctx_lat = jnp.concatenate(ctx_parts, axis=0)

    res["bwuv"].wait()
    ctx = jnp.dot(ctx_lat, bwuv_v[...].reshape(dc, hd),
                  preferred_element_type=f32)
    ctx = jnp.where(diag, ctx, 0.0).astype(bf16)
    res["bwo"].wait()
    t = jnp.dot(ctx, bwo_v[...], preferred_element_type=f32)
    for b in range(nb):
        ob = jnp.sum(t[b * nh:(b + 1) * nh], axis=0, keepdims=True)
        out_ref[b, :, pl.ds(d_model, bwo_v.shape[1])] = ob.astype(out_ref.dtype)

    res["ax"].wait()
    xa = rows_of(ax_v)
    res["awq"].wait()
    qa = jnp.dot(xa, awq_v[...], preferred_element_type=f32)
    qa = qa.astype(bf16)
    for h in range(nh):
        q_scr[h] = qa[:, h * dh:(h + 1) * dh]

    row_o = lax.broadcasted_iota(jnp.int32, (8, dh), 0)

    def attend(i, q):
        slot = lax.rem(i, depth)
        nxt = i + depth
        k_copy(i, slot).wait()
        s = lax.dot_general(q, kbuf[slot], _NT, preferred_element_type=f32)

        @pl.when(nxt < nsteps)
        def _():
            k_copy(nxt, slot).start()

        s = s * scale
        m = jnp.max(s, axis=1, keepdims=True)
        p = jnp.exp(s - m)
        l = jnp.sum(p, axis=1, keepdims=True)
        p = p.astype(bf16)
        v_copy(i, slot).wait()
        o = jnp.dot(p, vbuf[slot], preferred_element_type=f32)

        @pl.when(nxt < nsteps)
        def _():
            v_copy(nxt, slot).start()

        return o / l

    res["awo"].wait()

    def head_body(h, acc):
        q = q_scr[h]
        o = jnp.zeros((8, dh), f32)
        for b in range(nb):
            o = jnp.where(row_o == b, attend(h * nb + b, q), o)
        wo = awo_v[pl.ds(pl.multiple_of(h * dh, dh), dh), :]
        return acc + jnp.dot(o.astype(bf16), wo, preferred_element_type=f32)

    acc = lax.fori_loop(0, nh, head_body,
                        jnp.zeros((8, awo_v.shape[1]), f32))
    for b in range(nb):
        out_ref[b, :, pl.ds(0, awo_v.shape[1])] = (
            acc[b:b + 1].astype(out_ref.dtype))


@jax.jit
def pallas_concat_heads__gqa_block_cached__compressed_kv_cla__decode_kernel(
    A_x: jax.Array,
    A_k_cache: jax.Array,
    A_v_cache: jax.Array,
    A_wq: jax.Array,
    A_wo: jax.Array,
    B_x: jax.Array,
    B_c_kv: jax.Array,
    B_w_q: jax.Array,
    B_w_uk: jax.Array,
    B_w_uv: jax.Array,
    B_w_o: jax.Array,
):
    nb, sq, d_model = A_x.shape
    _, nh, sk, dh = A_k_cache.shape
    assert sq == 1 and A_wq.shape == (d_model, nh * dh)
    h_b, d_b, m_b = B_w_o.shape
    assert B_w_q.shape[1:] == (nh, dh) and (h_b, d_b) == (nh, dh)
    B_w_o2 = B_w_o.reshape(h_b * d_b, m_b)
    bf16 = jnp.bfloat16

    hbm = pl.BlockSpec(memory_space=pl.ANY)
    kernel = lambda *refs: _kernel(*refs, nb=nb, nh=nh, dh=dh, depth=DEPTH)
    return pl.pallas_call(
        kernel,
        out_shape=jax.ShapeDtypeStruct((nb, sq, A_wo.shape[1] + m_b), A_x.dtype),
        in_specs=[hbm] * 11,
        out_specs=pl.BlockSpec(memory_space=pltpu.VMEM),
        scratch_shapes=[
            pltpu.VMEM(A_x.shape, bf16),
            pltpu.VMEM(B_x.shape, bf16),
            pltpu.VMEM(A_wq.shape, bf16),
            pltpu.VMEM(A_wo.shape, bf16),
            pltpu.VMEM(B_c_kv.shape, bf16),
            pltpu.VMEM(B_w_q.shape, bf16),
            pltpu.VMEM(B_w_uk.shape, bf16),
            pltpu.VMEM(B_w_uv.shape, bf16),
            pltpu.VMEM(B_w_o2.shape, bf16),
            pltpu.VMEM((DEPTH, sk, dh), bf16),
            pltpu.VMEM((DEPTH, sk, dh), bf16),
            pltpu.VMEM((nh, 8, dh), bf16),
            pltpu.SemaphoreType.DMA((8 + nb,)),
            pltpu.SemaphoreType.DMA((DEPTH,)),
            pltpu.SemaphoreType.DMA((DEPTH,)),
        ],
        compiler_params=pltpu.CompilerParams(vmem_limit_bytes=VMEM_LIMIT),
    )(A_x, A_k_cache, A_v_cache, A_wq, A_wo,
      B_x, B_c_kv, B_w_q, B_w_uk, B_w_uv, B_w_o2)
```

```python
import contextlib
import jax
import jax.numpy as jnp
from jax import lax
import jax.experimental.pallas as pl
import jax.experimental.pallas.tpu as pltpu

DEPTH = 2
LOOKAHEAD = 3
VMEM_LIMIT = 100 * 1024 * 1024
SCOPES = False

_NT = (((1,), (1,)), ((), ()))

PIECE_BYTES = 57 * 1024


def scope(name):
    return jax.named_scope(name) if SCOPES else contextlib.nullcontext()


def _split(total, unit, n):
    q, r = divmod(total // unit, n)
    sizes = [(q + 1) * unit] * r + [q * unit] * (n - r)
    out, pos = [], 0
    for s in sizes:
        out.append(pl.ds(pos, s))
        pos += s
    return out


def _pieces(shape, itemsize):
    total = itemsize
    for s in shape:
        total *= s
    n = 2 * max(1, round(total / PIECE_BYTES / 2))
    if total <= PIECE_BYTES:
        return [(pl.ds(0, shape[0]),)]
    if len(shape) == 3:
        return [(s,) for s in _split(shape[0], 1, n)]
    rows, cols = shape
    if 16 * cols * itemsize <= PIECE_BYTES:
        return [(s,) for s in _split(rows, 16, n)]
    per = n // (rows // 16)
    return [(pl.ds(r, 16), c) for r in range(0, rows, 16)
            for c in _split(cols, 128, per + 1 if per % 2 else per)]


def _kernel(
    ax_hbm, k_hbm, v_hbm, awq_hbm, awo_hbm,
    bx_hbm, ckv_hbm, bwq_hbm, bwuk_hbm, bwuv_hbm, bwo_hbm,
    out_ref,
    ax_v, bx_v, awq_v, awo_v, ckv_v, bwq_v, bwuk_v, bwuv_v, bwo_v,
    kbuf, vbuf, q_scr, rsem, ksem, vsem,
    *, nb, nh, dh, depth, nchunk,
):
    f32, bf16 = jnp.float32, jnp.bfloat16
    nsteps = nb * nh
    d_model = ax_v.shape[-1]
    sk, dc = ckv_v.shape[1:]
    hd = nh * dh
    scale = dh ** -0.5

    def start_pieces(src, dst, sem, pieces):
        for j, idx in enumerate(pieces):
            pltpu.make_async_copy(src.at[idx], dst.at[idx], sem).start(
                priority=j % 2)

    def wait_all(dst, sem):
        pltpu.make_async_copy(dst, dst, sem).wait()

    kv_pieces = _pieces(kbuf.shape[1:], 2)

    def k_start(i, slot):
        start_pieces(k_hbm.at[i % nb, i // nb], kbuf.at[slot], ksem.at[slot],
                     kv_pieces)

    def v_start(i, slot):
        start_pieces(v_hbm.at[i % nb, i // nb], vbuf.at[slot], vsem.at[slot],
                     kv_pieces)

    row8 = lax.broadcasted_iota(jnp.int32, (8, d_model), 0)

    def rows_of(x_v):
        x = x_v[...].astype(f32)
        out = jnp.zeros((8, d_model), f32)
        for b in range(nb):
            out = jnp.where(row8 == b, x[b:b + 1], out)
        return out.astype(bf16)

    rows = lax.broadcasted_iota(jnp.int32, (nb * nh, hd), 0)
    lanes = lax.broadcasted_iota(jnp.int32, (nb * nh, hd), 1)
    diag = (rows % nh) == (lanes // dh)

    st = {}
    units = []

    def halves(name, src, dst, compute):
        n = dst.shape[0] // 2
        for j in range(2):
            sl = pl.ds(j * n, n)
            units.append((f"{name}{j}", src.at[sl], dst.at[sl],
                          (lambda j=j, ref=dst.at[sl]: compute(j, ref))
                          if compute else None))

    def c_bx():
        st["xb"] = rows_of(bx_v)

    def c_ax():
        st["xa"] = rows_of(ax_v)

    units.append(("bx", bx_hbm, bx_v, c_bx))
    units.append(("ax", ax_hbm, ax_v, c_ax))

    def c_bwq(j, w):
        n = w.shape[0]
        part = jnp.dot(st["xb"][:, j * n:(j + 1) * n], w[...].reshape(n, hd),
                       preferred_element_type=f32)
        if j == 0:
            st["qb"] = part
            return
        qb = (st["qb"] + part).astype(bf16).astype(f32)
        q_bd = jnp.concatenate(
            [jnp.broadcast_to(qb[b:b + 1], (nh, hd)) for b in range(nb)], axis=0)
        st["q_bd"] = jnp.where(diag, q_bd, 0.0).astype(bf16)

    halves("bwq", bwq_hbm, bwq_v, c_bwq)

    def c_bwuk(j, w):
        ql = lax.dot_general(st["q_bd"], w[...].reshape(w.shape[0], hd), _NT,
                             preferred_element_type=f32)
        st[f"ql{j}"] = (ql * scale).astype(bf16)
        if j == 1:
            st["qlat"] = jnp.concatenate([st["ql0"], st["ql1"]], axis=1)

    halves("bwuk", bwuk_hbm, bwuk_v, c_bwuk)

    ck = sk // nchunk

    def c_ckv(b, j, c_ref):
        ckv = c_ref[...]
        s = lax.dot_general(st["qlat"][b * nh:(b + 1) * nh], ckv, _NT,
                            preferred_element_type=f32)
        m = jnp.max(s, axis=1, keepdims=True)
        if j > 0:
            m = jnp.maximum(m, st["m"])
        p = jnp.exp(s - m)
        l = jnp.sum(p, axis=1, keepdims=True)
        acc = jnp.dot(p.astype(bf16), ckv, preferred_element_type=f32)
        if j > 0:
            alpha = jnp.exp(st["m"] - m)
            l = l + alpha * st["l"]
            acc = acc + alpha * st["acc"]
        st["m"], st["l"], st["acc"] = m, l, acc
        if j == nchunk - 1:
            st[f"ctx{b}"] = (acc / l).astype(bf16)

    for b in range(nb):
        for j in range(nchunk):
            sl = pl.ds(j * ck, ck)
            units.append((f"ckv{b}{j}", ckv_hbm.at[b, sl], ckv_v.at[b, sl],
                          lambda b=b, j=j, r=ckv_v.at[b, sl]: c_ckv(b, j, r)))

    def c_bwuv(j, w):
        n = w.shape[0]
        if j == 0:
            st["ctx_lat"] = jnp.concatenate(
                [st[f"ctx{b}"] for b in range(nb)], axis=0)
        part = jnp.dot(st["ctx_lat"][:, j * n:(j + 1) * n], w[...].reshape(n, hd),
                       preferred_element_type=f32)
        if j == 0:
            st["ctx"] = part
        else:
            st["ctx"] = jnp.where(diag, st["ctx"] + part, 0.0).astype(bf16)

    halves("bwuv", bwuv_hbm, bwuv_v, c_bwuv)

    def c_bwo(j, w):
        n = w.shape[0]
        part = jnp.dot(st["ctx"][:, j * n:(j + 1) * n], w[...],
                       preferred_element_type=f32)
        if j == 0:
            st["t"] = part
            return
        t = st["t"] + part
        for b in range(nb):
            ob = jnp.sum(t[b * nh:(b + 1) * nh], axis=0, keepdims=True)
            out_ref[b:b + 1, pl.ds(d_model, t.shape[1])] = ob.astype(out_ref.dtype)

    halves("bwo", bwo_hbm, bwo_v, c_bwo)

    def c_awq(j, w):
        n = w.shape[0]
        part = jnp.dot(st["xa"][:, j * n:(j + 1) * n], w[...],
                       preferred_element_type=f32)
        if j == 0:
            st["qa"] = part
            return
        qa = (st["qa"] + part).astype(bf16)
        for h in range(nh):
            q_scr[h] = qa[:, h * dh:(h + 1) * dh]

    halves("awq", awq_hbm, awq_v, c_awq)
    halves("awo", awo_hbm, awo_v, None)

    starts = []
    for n, (name, src, dst, _) in enumerate(units):
        starts.append(lambda name=name, src=src, dst=dst, n=n: start_pieces(
            src, dst, rsem.at[n], _pieces(dst.shape, 2)))
    for i in range(depth):
        starts.append(lambda i=i: k_start(i, i))
        starts.append(lambda i=i: v_start(i, i))

    issued = 0
    for n, (name, src, dst, compute) in enumerate(units):
        target = min(len(starts), n + 1 + LOOKAHEAD)
        with scope(f"start_upto_{target}"):
            while issued < target:
                starts[issued]()
                issued += 1
        with scope("wait_" + name):
            wait_all(dst, rsem.at[n])
        if compute is not None:
            with scope("c_" + name):
                compute()
    while issued < len(starts):
        starts[issued]()
        issued += 1

    row_o = lax.broadcasted_iota(jnp.int32, (8, dh), 0)

    def attend(i, q):
        slot = lax.rem(i, depth)
        nxt = i + depth
        wait_all(kbuf.at[slot], ksem.at[slot])
        s = lax.dot_general(q, kbuf[slot], _NT, preferred_element_type=f32)

        @pl.when(nxt < nsteps)
        def _():
            k_start(nxt, slot)

        s = s * scale
        m = jnp.max(s, axis=1, keepdims=True)
        p = jnp.exp(s - m)
        l = jnp.sum(p, axis=1, keepdims=True)
        p = p.astype(bf16)
        wait_all(vbuf.at[slot], vsem.at[slot])
        o = jnp.dot(p, vbuf[slot], preferred_element_type=f32)

        @pl.when(nxt < nsteps)
        def _():
            v_start(nxt, slot)

        return o / l

    def head_body(h, acc):
        q = q_scr[h]
        o = jnp.zeros((8, dh), f32)
        for b in range(nb):
            o = jnp.where(row_o == b, attend(h * nb + b, q), o)
        wo = awo_v[pl.ds(pl.multiple_of(h * dh, dh), dh), :]
        return acc + jnp.dot(o.astype(bf16), wo, preferred_element_type=f32)

    with scope("loop"):
        acc = lax.fori_loop(0, nh, head_body,
                            jnp.zeros((8, awo_v.shape[1]), f32))
    for b in range(nb):
        out_ref[b:b + 1, pl.ds(0, awo_v.shape[1])] = (
            acc[b:b + 1].astype(out_ref.dtype))


@jax.jit
def pallas_concat_heads__gqa_block_cached__compressed_kv_cla__decode_kernel(
    A_x: jax.Array,
    A_k_cache: jax.Array,
    A_v_cache: jax.Array,
    A_wq: jax.Array,
    A_wo: jax.Array,
    B_x: jax.Array,
    B_c_kv: jax.Array,
    B_w_q: jax.Array,
    B_w_uk: jax.Array,
    B_w_uv: jax.Array,
    B_w_o: jax.Array,
):
    nb, sq, d_model = A_x.shape
    _, nh, sk, dh = A_k_cache.shape
    assert sq == 1 and A_wq.shape == (d_model, nh * dh)
    h_b, d_b, m_b = B_w_o.shape
    assert B_w_q.shape[1:] == (nh, dh) and (h_b, d_b) == (nh, dh)
    B_w_o2 = B_w_o.reshape(h_b * d_b, m_b)
    bf16 = jnp.bfloat16
    nchunk = 4

    hbm = pl.BlockSpec(memory_space=pl.ANY)
    kernel = lambda *refs: _kernel(*refs, nb=nb, nh=nh, dh=dh, depth=DEPTH, nchunk=nchunk)
    out = pl.pallas_call(
        kernel,
        out_shape=jax.ShapeDtypeStruct((nb, A_wo.shape[1] + m_b), A_x.dtype),
        in_specs=[hbm] * 11,
        out_specs=pl.BlockSpec(memory_space=pltpu.VMEM),
        scratch_shapes=[
            pltpu.VMEM((nb, d_model), bf16),
            pltpu.VMEM((nb, B_x.shape[2]), bf16),
            pltpu.VMEM(A_wq.shape, bf16),
            pltpu.VMEM(A_wo.shape, bf16),
            pltpu.VMEM(B_c_kv.shape, bf16),
            pltpu.VMEM(B_w_q.shape, bf16),
            pltpu.VMEM(B_w_uk.shape, bf16),
            pltpu.VMEM(B_w_uv.shape, bf16),
            pltpu.VMEM(B_w_o2.shape, bf16),
            pltpu.VMEM((DEPTH, sk, dh), bf16),
            pltpu.VMEM((DEPTH, sk, dh), bf16),
            pltpu.VMEM((nh, 8, dh), bf16),
            pltpu.SemaphoreType.DMA((12 + nb * nchunk,)),
            pltpu.SemaphoreType.DMA((DEPTH,)),
            pltpu.SemaphoreType.DMA((DEPTH,)),
        ],
        compiler_params=pltpu.CompilerParams(vmem_limit_bytes=VMEM_LIMIT),
    )(A_x.reshape(nb, d_model), A_k_cache, A_v_cache, A_wq, A_wo,
      B_x.reshape(nb, B_x.shape[2]), B_c_kv, B_w_q, B_w_uk, B_w_uv, B_w_o2)
    return out.reshape(nb, sq, out.shape[1])
```

```python
import jax
import jax.numpy as jnp
from jax import lax
import jax.experimental.pallas as pl
import jax.experimental.pallas.tpu as pltpu

UNIT_BYTES = 2 * 1024 * 1024
N_STREAMS = 8
N_ROUNDS = 8
LOOKAHEAD = 3
VMEM_LIMIT = 100 * 1024 * 1024

_NT = (((1,), (1,)), ((), ()))


def _pieces(shape):
    total = 2
    for s in shape:
        total *= s
    if total != UNIT_BYTES:
        return [((pl.ds(0, shape[0]),), 0)]
    nblk = N_STREAMS * N_ROUNDS
    out = []
    for j in reversed(range(N_ROUNDS)):
        for k in (t ^ 1 for t in range(N_STREAMS)):
            blk = k * N_ROUNDS + j
            if shape[0] % (16 * nblk) == 0 or len(shape) == 3:
                rows = shape[0] // nblk
                idx = (pl.ds(blk * rows, rows),)
            else:
                per = 16 * nblk // shape[0]
                cols = shape[1] // per
                idx = (pl.ds(16 * (blk // per), 16),
                       pl.ds(cols * (blk % per), cols))
            out.append((idx, 1 - k % 2))
    return out


def _kernel(
    ax_hbm, k_hbm, v_hbm, awq_hbm, awo_hbm,
    bx_hbm, ckv_hbm, bwq_hbm, bwuk_hbm, bwuv_hbm, bwo_hbm,
    out_ref,
    ax_v, bx_v, awq_v, awo_v, ckv_v, bwq_v, bwuk_v, bwuv_v, bwo_v,
    kbuf, vbuf, q_scr, rsem, ksem, vsem,
):
    f32, bf16 = jnp.float32, jnp.bfloat16
    nb, d_model = ax_v.shape
    nh, _, dh = q_scr.shape
    _, sk, dc = ckv_v.shape
    hd = nh * dh
    scale = dh ** -0.5

    def start_unit(src, dst, sem):
        for idx, prio in _pieces(dst.shape):
            pltpu.make_async_copy(src.at[idx], dst.at[idx], sem).start(priority=prio)

    def wait_unit(dst, sem):
        pltpu.make_async_copy(dst, dst, sem).wait()

    def k_start(b, h):
        start_unit(k_hbm.at[b, h], kbuf.at[b], ksem.at[b])

    def v_start(b, h):
        start_unit(v_hbm.at[b, h], vbuf.at[b], vsem.at[b])

    row8 = lax.broadcasted_iota(jnp.int32, (8, d_model), 0)

    def rows_of(x_v):
        x = x_v[...].astype(f32)
        out = jnp.zeros((8, d_model), f32)
        for b in range(nb):
            out = jnp.where(row8 == b, x[b:b + 1], out)
        return out.astype(bf16)

    rows = lax.broadcasted_iota(jnp.int32, (nb * nh, hd), 0)
    lanes = lax.broadcasted_iota(jnp.int32, (nb * nh, hd), 1)
    diag = (rows % nh) == (lanes // dh)

    units = []
    st = {}

    def add_rows(src, dst, compute):
        n = dst.size * 2 // UNIT_BYTES
        step = dst.shape[0] // n
        for j in range(n):
            sl = pl.ds(j * step, step)
            fn = None
            if compute is not None:
                fn = lambda j=j, ref=dst.at[sl]: compute(j, n, ref)
            units.append((src.at[sl], dst.at[sl], fn))

    def accumulate(key, j, part):
        st[key] = part if j == 0 else st[key] + part
        return st[key]

    def c_bx():
        st["xb"] = rows_of(bx_v)

    def c_ax():
        st["xa"] = rows_of(ax_v)

    units.append((bx_hbm, bx_v, c_bx))
    units.append((ax_hbm, ax_v, c_ax))

    def c_bwq(j, n, w):
        m = w.shape[0]
        qb = accumulate("qb", j, jnp.dot(
            st["xb"][:, j * m:(j + 1) * m], w[...].reshape(m, hd),
            preferred_element_type=f32))
        if j == n - 1:
            qb = qb.astype(bf16).astype(f32)
            q_bd = jnp.concatenate(
                [jnp.broadcast_to(qb[b:b + 1], (nh, hd)) for b in range(nb)],
                axis=0)
            st["q_bd"] = jnp.where(diag, q_bd, 0.0).astype(bf16)

    add_rows(bwq_hbm, bwq_v, c_bwq)

    def c_bwuk(j, n, w):
        ql = lax.dot_general(st["q_bd"], w[...].reshape(w.shape[0], hd), _NT,
                             preferred_element_type=f32)
        st["ql", j] = (ql * scale).astype(bf16)
        if j == n - 1:
            st["qlat"] = jnp.concatenate([st["ql", i] for i in range(n)], axis=1)

    add_rows(bwuk_hbm, bwuk_v, c_bwuk)

    def c_ckv(b, j, n, c_ref):
        ckv = c_ref[...]
        s = lax.dot_general(st["qlat"][b * nh:(b + 1) * nh], ckv, _NT,
                            preferred_element_type=f32)
        m = jnp.max(s, axis=1, keepdims=True)
        if j > 0:
            m = jnp.maximum(m, st["m"])
        p = jnp.exp(s - m)
        l = jnp.sum(p, axis=1, keepdims=True)
        acc = jnp.dot(p.astype(bf16), ckv, preferred_element_type=f32)
        if j > 0:
            alpha = jnp.exp(st["m"] - m)
            l = l + alpha * st["l"]
            acc = acc + alpha * st["acc"]
        st["m"], st["l"], st["acc"] = m, l, acc
        if j == n - 1:
            st["ctx", b] = (acc / l).astype(bf16)

    for b in range(nb):
        add_rows(ckv_hbm.at[b], ckv_v.at[b],
                 lambda j, n, ref, b=b: c_ckv(b, j, n, ref))

    def c_bwuv(j, n, w):
        m = w.shape[0]
        if j == 0:
            st["ctx_lat"] = jnp.concatenate(
                [st["ctx", b] for b in range(nb)], axis=0)
        ctx = accumulate("ctx_full", j, jnp.dot(
            st["ctx_lat"][:, j * m:(j + 1) * m], w[...].reshape(m, hd),
            preferred_element_type=f32))
        if j == n - 1:
            st["ctx_bd"] = jnp.where(diag, ctx, 0.0).astype(bf16)

    add_rows(bwuv_hbm, bwuv_v, c_bwuv)

    def c_bwo(j, n, w):
        m = w.shape[0]
        t = accumulate("t", j, jnp.dot(
            st["ctx_bd"][:, j * m:(j + 1) * m], w[...],
            preferred_element_type=f32))
        if j == n - 1:
            for b in range(nb):
                ob = jnp.sum(t[b * nh:(b + 1) * nh], axis=0, keepdims=True)
                out_ref[b:b + 1, pl.ds(awo_v.shape[1], t.shape[1])] = (
                    ob.astype(out_ref.dtype))

    add_rows(bwo_hbm, bwo_v, c_bwo)

    def c_awq(j, n, w):
        m = w.shape[0]
        qa = accumulate("qa", j, jnp.dot(
            st["xa"][:, j * m:(j + 1) * m], w[...],
            preferred_element_type=f32))
        if j == n - 1:
            qa = qa.astype(bf16)
            for h in range(nh):
                q_scr[h] = qa[:, h * dh:(h + 1) * dh]

    add_rows(awq_hbm, awq_v, c_awq)
    add_rows(awo_hbm, awo_v, None)

    starts = [lambda n=n, u=u: start_unit(u[0], u[1], rsem.at[n])
              for n, u in enumerate(units)]
    for b in range(nb):
        starts.append(lambda b=b: k_start(b, 0))
        starts.append(lambda b=b: v_start(b, 0))

    issued = 0
    for n, (_, dst, compute) in enumerate(units):
        while issued < min(len(starts), n + 1 + LOOKAHEAD):
            starts[issued]()
            issued += 1
        wait_unit(dst, rsem.at[n])
        if compute is not None:
            compute()
    while issued < len(starts):
        starts[issued]()
        issued += 1

    row_o = lax.broadcasted_iota(jnp.int32, (8, dh), 0)

    def attend(b, h, q):
        wait_unit(kbuf.at[b], ksem.at[b])
        s = lax.dot_general(q, kbuf[b], _NT, preferred_element_type=f32)

        @pl.when(h + 1 < nh)
        def _():
            k_start(b, h + 1)

        s = s * scale
        m = jnp.max(s, axis=1, keepdims=True)
        p = jnp.exp(s - m)
        l = jnp.sum(p, axis=1, keepdims=True)
        p = p.astype(bf16)
        wait_unit(vbuf.at[b], vsem.at[b])
        o = jnp.dot(p, vbuf[b], preferred_element_type=f32)

        @pl.when(h + 1 < nh)
        def _():
            v_start(b, h + 1)

        return o / l

    def head_body(h, acc):
        q = q_scr[h]
        o = jnp.zeros((8, dh), f32)
        for b in range(nb):
            o = jnp.where(row_o == b, attend(b, h, q), o)
        wo = awo_v[pl.ds(pl.multiple_of(h * dh, dh), dh), :]
        return acc + jnp.dot(o.astype(bf16), wo, preferred_element_type=f32)

    acc = lax.fori_loop(0, nh, head_body,
                        jnp.zeros((8, awo_v.shape[1]), f32))
    for b in range(nb):
        out_ref[b:b + 1, pl.ds(0, awo_v.shape[1])] = (
            acc[b:b + 1].astype(out_ref.dtype))


@jax.jit
def pallas_concat_heads__gqa_block_cached__compressed_kv_cla__decode_kernel(
    A_x: jax.Array,
    A_k_cache: jax.Array,
    A_v_cache: jax.Array,
    A_wq: jax.Array,
    A_wo: jax.Array,
    B_x: jax.Array,
    B_c_kv: jax.Array,
    B_w_q: jax.Array,
    B_w_uk: jax.Array,
    B_w_uv: jax.Array,
    B_w_o: jax.Array,
):
    nb, sq, d_model = A_x.shape
    _, nh, sk, dh = A_k_cache.shape
    h_b, d_b, m_b = B_w_o.shape
    assert sq == 1 and A_wq.shape == (d_model, nh * dh)
    assert B_w_q.shape[1:] == (nh, dh) and (h_b, d_b) == (nh, dh)
    assert B_x.shape == A_x.shape
    bf16 = jnp.bfloat16

    B_w_o2 = B_w_o.reshape(h_b * d_b, m_b)
    resident = (A_wq, A_wo, B_c_kv, B_w_q, B_w_uk, B_w_uv, B_w_o2)
    n_units = 2 + sum(a.size * 2 // UNIT_BYTES for a in resident)

    hbm = pl.BlockSpec(memory_space=pl.ANY)
    out = pl.pallas_call(
        _kernel,
        out_shape=jax.ShapeDtypeStruct((nb, A_wo.shape[1] + m_b), A_x.dtype),
        in_specs=[hbm] * 11,
        out_specs=pl.BlockSpec(memory_space=pltpu.VMEM),
        scratch_shapes=[
            pltpu.VMEM((nb, d_model), bf16),
            pltpu.VMEM((nb, d_model), bf16),
            pltpu.VMEM(A_wq.shape, bf16),
            pltpu.VMEM(A_wo.shape, bf16),
            pltpu.VMEM(B_c_kv.shape, bf16),
            pltpu.VMEM(B_w_q.shape, bf16),
            pltpu.VMEM(B_w_uk.shape, bf16),
            pltpu.VMEM(B_w_uv.shape, bf16),
            pltpu.VMEM(B_w_o2.shape, bf16),
            pltpu.VMEM((nb, sk, dh), bf16),
            pltpu.VMEM((nb, sk, dh), bf16),
            pltpu.VMEM((nh, 8, dh), bf16),
            pltpu.SemaphoreType.DMA((n_units,)),
            pltpu.SemaphoreType.DMA((nb,)),
            pltpu.SemaphoreType.DMA((nb,)),
        ],
        compiler_params=pltpu.CompilerParams(vmem_limit_bytes=VMEM_LIMIT),
    )(A_x.reshape(nb, d_model), A_k_cache, A_v_cache, A_wq, A_wo,
      B_x.reshape(nb, d_model), B_c_kv, B_w_q, B_w_uk, B_w_uv, B_w_o2)
    return out.reshape(nb, sq, out.shape[1])
```
